```python
import os as _os
_os.environ.setdefault("JAX_PLATFORMS", "cpu")
import jax
import jax.numpy as jnp

def _softmax(x, axis=-1):
    return jax.nn.softmax(x, axis=axis)
def _gelu(x):
    return jax.nn.gelu(x, approximate=True)
def _silu(x):
    return jax.nn.silu(x)
def _sigmoid(x):
    return jax.nn.sigmoid(x)
def _layernorm(x, axis=-1, eps=1e-5):
    m = jnp.mean(x, axis=axis, keepdims=True)
    v = jnp.var(x, axis=axis, keepdims=True)
    return (x - m) / jnp.sqrt(v + eps)
def _scatter_add(tgt, idx, src, axis=0):
    return tgt.at[idx].add(src)
def _segment_sum(src, seg, n):
    return jax.ops.segment_sum(src, seg, n)
class _Rng:
    def __init__(self, key):
        self._k = key
    def _next(self):
        self._k, sub = jax.random.split(self._k)
        return sub
    def normal(self, shape):
        return jax.random.normal(self._next(), shape, dtype=jnp.bfloat16)
    def randint(self, lo, hi, shape):
        return jax.random.randint(self._next(), shape, lo, hi, dtype=jnp.int32)
    def uniform(self, shape, lo=0.0, hi=1.0):
        return jax.random.uniform(self._next(), shape, jnp.bfloat16, lo, hi)
    def permutation(self, n):
        return jax.random.permutation(self._next(), n)


kernel_name = 'parallel_sum__ssm_conv_h3__dense_activation_silu__prompt'

def setup_inputs():
    _rng = _Rng(jax.random.key(int.from_bytes(__import__("os").urandom(4), "little")))
    _w = (lambda a: (lambda t: t.astype(jnp.bfloat16) if jnp.issubdtype(t.dtype, jnp.floating) else t)(jnp.asarray(a)))
    def _A_setup():
        B, S, D = 1, 2048, 448
        ks = 4
        return {
            "q": _w((lambda *s: _rng.normal(s) * 0.05)(B, S, D)),
            "k": _w((lambda *s: _rng.normal(s) * 0.2)(B, S, D)),
            "v": _w((lambda *s: _rng.normal(s) * 0.2)(B, S, D)),
            "shift_k": _w((lambda *s: _rng.normal(s) * 0.2)(D, ks) * 0.5),
            "ssm_k": _w((lambda *s: _rng.normal(s) * 0.2)(D, S) * (1.0 / S ** 0.5)),
            "ssm_D": _w((lambda *s: _rng.normal(s) * 0.2)(D)),
        }
    _A_in = _A_setup()

    def _B_setup():
        B, S, D, F = 1, 2048, 448, 1792
        return {
            "x": _w((lambda *s: _rng.normal(s) * 0.05)(B, S, D)),
            "w1": _w((lambda *s: _rng.normal(s) * 0.05)(D, F) * (D ** -0.5)),
            "w2": _w((lambda *s: _rng.normal(s) * 0.05)(F, D) * (F ** -0.5)),
        }
    _B_in = _B_setup()

    return {
        "A_q": _A_in["q"],
        "A_k": _A_in["k"],
        "A_v": _A_in["v"],
        "A_shift_k": _A_in["shift_k"],
        "A_ssm_k": _A_in["ssm_k"],
        "A_ssm_D": _A_in["ssm_D"],
        "B_x": _B_in["x"],
        "B_w1": _B_in["w1"],
        "B_w2": _B_in["w2"],
    }

def reference(A_q, A_k, A_v, A_shift_k, A_ssm_k, A_ssm_D, B_x, B_w1, B_w2):
    def _A_ref(q, k, v, shift_k, ssm_k, ssm_D):
        B, S, D = q.shape
        ks = shift_k.shape[-1]
        k_pad = jnp.pad(k, ((0, 0), (ks - 1, 0), (0, 0)))
        k_shift = jnp.zeros_like(k)
        for t in range(ks):
            k_shift = k_shift + k_pad[:, t:t + S, :] * shift_k[:, ks - 1 - t][None, None, :]
        kv = k_shift * v
        L = 2 * S
        kv_pad = jnp.pad(kv, ((0, 0), (0, S), (0, 0)))
        kf_pad = jnp.pad(ssm_k, ((0, 0), (0, S)))
        kv_f = (lambda x, axes=(-2,-1): jnp.fft.rfft2(x.astype(jnp.float32), axes=axes))(kv_pad[:, None, :, :], axes=(1, 2))
        kf_f = (lambda x, axes=(-2,-1): jnp.fft.rfft2(x.astype(jnp.float32), axes=axes))(kf_pad[:, None, :], axes=(1, 2))
        kf_f = (lambda x, *d: x.transpose(*d))(kf_f, 1, 2, 0)
        y_f = kv_f * kf_f[None, :, :, :]
        y = (lambda x, s, axes=(-2,-1): jnp.fft.irfft2(x, s=s, axes=axes).astype(jnp.bfloat16))(y_f, (1, L), axes=(1, 2))[:, 0, :S, :]
        y = y + kv * ssm_D[None, None, :]
        return q * y

    def _B_ref(x, w1, w2):
        h = jnp.einsum("bsd,df->bsf", x, w1)
        h = _silu(h)
        out = jnp.einsum("bsf,fd->bsd", h, w2)
        return out

    x = A_q
    xn = _layernorm(x, axis=-1)
    return x + _A_ref(xn, A_k, A_v, A_shift_k, A_ssm_k, A_ssm_D) + _B_ref(xn, B_w1, B_w2)
```

```python
import numpy as np
import jax
import jax.numpy as jnp
import jax.experimental.pallas as pl
import jax.experimental.pallas.tpu as pltpu

S, D, F = 2048, 448, 1792
NB = S // 128


def _consts():
    b = np.arange(128, dtype=np.float64)[:, None]
    f = np.arange(128, dtype=np.float64)[None, :]
    th = 2.0 * np.pi * b * (f - 0.25) / 128.0
    T = np.concatenate([np.cos(th), -np.sin(th)], axis=1)
    G = T.T / 128.0
    return T.astype(jnp.bfloat16), G.astype(jnp.bfloat16)


def kernel(x_ref, k_ref, v_ref, sh_ref, sk_ref, d_ref, w1_ref, w2t_ref, t_ref, g_ref, o_ref,
           w1t_ref, xn_ref, wb_ref, kv_ref, h_ref, xh_ref, kh_ref, wv_ref, acc_ref):
    f32, bf16 = jnp.float32, jnp.bfloat16
    sh = sh_ref[...].astype(f32)
    dd = d_ref[...].astype(f32).reshape(1, D)
    p = jnp.concatenate([sh, dd, jnp.zeros((3, D), f32)], axis=0)
    p = jnp.concatenate([p, jnp.zeros((8, 64), f32)], axis=1)
    p = jnp.concatenate([p, jnp.zeros((120, 512), f32)], axis=0)
    pt = p.T
    for j in range(5):
        wb_ref[j] = jnp.broadcast_to(pt[0:D, j:j + 1], (D, 128))

    w1t_ref[...] = (w1_ref[...].astype(f32) * 0.5).astype(bf16).T

    for c in range(4):
        cs = slice(512 * c, 512 * (c + 1))
        x = x_ref[:, cs].astype(f32)
        m = jnp.sum(x, axis=0, keepdims=True) * (1.0 / D)
        xc = x - m
        var = jnp.sum(xc * xc, axis=0, keepdims=True) * (1.0 / D)
        xn_ref[:, cs] = (xc * jax.lax.rsqrt(var + 1e-5)).astype(bf16)

    for c in range(4):
        cs = slice(512 * c, 512 * (c + 1))
        h = jnp.dot(w1t_ref[...], xn_ref[:, cs], preferred_element_type=f32)
        h_ref[:, cs] = (h + h * jnp.tanh(h)).astype(bf16)

    lane = jax.lax.broadcasted_iota(jnp.int32, (D // 2, 128), 1)
    ku = pltpu.bitcast(k_ref[...], jnp.uint32)
    prev = [jnp.zeros((D // 2, 128), jnp.uint32)] * 3
    for a in range(NB):
        cs = slice(128 * a, 128 * (a + 1))
        kt = ku[:, cs]
        acc = pltpu.bitcast(kt, bf16).astype(f32) * wb_ref[0]
        cur = []
        for j in range(1, 4):
            r = pltpu.roll(kt, j, 1)
            cur.append(r)
            sel = jnp.where(lane < j, prev[j - 1], r)
            acc = acc + pltpu.bitcast(sel, bf16).astype(f32) * wb_ref[j]
        prev = cur
        kv_ref[:, cs] = (acc * v_ref[:, cs].astype(f32)).astype(bf16)

    T = t_ref[...]
    for a in range(NB):
        cs = slice(128 * a, 128 * (a + 1))
        r = jnp.dot(kv_ref[:, cs], T, preferred_element_type=f32)
        xr, xi = r[:, :128], r[:, 128:]
        xh_ref[0, a] = xr
        xh_ref[1, a] = xi
        xh_ref[2, a] = xr + xi
        r = jnp.dot(sk_ref[:, cs], T, preferred_element_type=f32)
        kr, ki = r[:, :128], r[:, 128:]
        if a == 0:
            kr = kr + wb_ref[4]
        kh_ref[0, a] = kr
        kh_ref[1, a] = ki - kr
        kh_ref[2, a] = kr + ki

    SB = 4
    for g in range(D // 8):
        rs = slice(8 * g, 8 * (g + 1))
        pre = pim = None
        for sb in range(0, NB, SB):
            S1 = [None] * SB
            S2 = [None] * SB
            S3 = [None] * SB
            for a in range(sb + SB):
                xr, xi, xs = xh_ref[0, a, rs], xh_ref[1, a, rs], xh_ref[2, a, rs]
                for i in range(SB):
                    c = sb + i - a
                    if c < 0:
                        continue
                    t1 = kh_ref[0, c, rs] * xs
                    t2 = kh_ref[1, c, rs] * xr
                    t3 = kh_ref[2, c, rs] * xi
                    S1[i] = t1 if S1[i] is None else S1[i] + t1
                    S2[i] = t2 if S2[i] is None else S2[i] + t2
                    S3[i] = t3 if S3[i] is None else S3[i] + t3
            for i in range(SB):
                re = S1[i] - S3[i]
                im = S1[i] + S2[i]
                if pre is None:
                    wr, wi = re, im
                else:
                    wr, wi = re + pim, im - pre
                pre, pim = re, im
                wv_ref[sb + i, 0, rs] = wr
                wv_ref[sb + i, 1, rs] = wi

    for c in range(4):
        cs = slice(512 * c, 512 * (c + 1))
        acc_ref[:, cs] = jnp.dot(w2t_ref[...], h_ref[:, cs], preferred_element_type=f32)

    G = g_ref[...]
    for s in range(NB):
        cs = slice(128 * s, 128 * (s + 1))
        lhs = jnp.concatenate([wv_ref[s, 0].astype(bf16), wv_ref[s, 1].astype(bf16)], axis=1)
        y = jnp.dot(lhs, G, preferred_element_type=f32)
        o = x_ref[:, cs].astype(f32) + xn_ref[:, cs].astype(f32) * y + acc_ref[:, cs]
        o_ref[:, cs] = o.astype(bf16)


def fn(A_q, A_k, A_v, A_shift_k, A_ssm_k, A_ssm_D, B_x, B_w1, B_w2):
    T, G = _consts()
    f32, bf16 = jnp.float32, jnp.bfloat16
    out = pl.pallas_call(
        kernel,
        out_shape=jax.ShapeDtypeStruct((D, S), bf16),
        scratch_shapes=[
            pltpu.VMEM((F, D), bf16),
            pltpu.VMEM((D, S), bf16),
            pltpu.VMEM((5, D, 128), f32),
            pltpu.VMEM((D, S), bf16),
            pltpu.VMEM((F, S), bf16),
            pltpu.VMEM((3, NB, D, 128), f32),
            pltpu.VMEM((3, NB, D, 128), f32),
            pltpu.VMEM((NB, 2, D, 128), f32),
            pltpu.VMEM((D, S), f32),
        ],
        compiler_params=pltpu.CompilerParams(vmem_limit_bytes=120 * 2**20),
    )(A_q[0].T, A_k[0].T, A_v[0].T, A_shift_k.T, A_ssm_k, A_ssm_D, B_w1, B_w2.T, T, G)
    return out.T[None]

@jax.jit
def pallas_parallel_sum__ssm_conv_h3__dense_activation_silu__prompt_kernel(
    A_q, A_k, A_v, A_shift_k, A_ssm_k, A_ssm_D, B_x, B_w1, B_w2):
    return fn(A_q, A_k, A_v, A_shift_k, A_ssm_k, A_ssm_D, B_x, B_w1, B_w2)
```

```python
import numpy as np
import jax
import jax.numpy as jnp
import jax.experimental.pallas as pl
import jax.experimental.pallas.tpu as pltpu

S, D, F = 2048, 448, 1792
NB = S // 128
NG = D // 8

EGAP = 448
N_PRE = 5
TIES = 1
OG = 1
LOOPS = 2
X0 = 4


def _consts():
    b = np.arange(128, dtype=np.float64)[:, None]
    f = np.arange(128, dtype=np.float64)[None, :]
    th = 2.0 * np.pi * b * (f - 0.25) / 128.0
    T = np.concatenate([np.cos(th), -np.sin(th)], axis=1)
    G = T.T / 64.0
    return T.astype(jnp.bfloat16), G.astype(jnp.bfloat16)


def kernel(x_hbm, k_hbm, v_hbm, sh_hbm, sk_hbm, d_hbm, w1_hbm, w2t_hbm, t_hbm, g_hbm, z_hbm, o_hbm,
           x_ref, k_ref, v_ref, sh_ref, sk_ref, d_ref, w1_ref, w2t_ref, t_ref, g_ref, o_ref,
           w1t_ref, xn_ref, wb_ref, h_ref, xh_ref, kh_ref, wv_ref, acc_ref, z_ref, sems):
    f32, bf16, u32 = jnp.float32, jnp.bfloat16, jnp.uint32

    def cp(src, dst, i):
        return pltpu.make_async_copy(src, dst, sems.at[i])

    c0 = 128 * X0
    cp_w1 = cp(w1_hbm, w1_ref, 0)
    cp_x0 = cp(x_hbm.at[:, 0:c0], x_ref.at[:, 0:c0], 1)
    cp_c = [cp(sh_hbm, sh_ref, 2), cp(d_hbm, d_ref, 3), cp(t_hbm, t_ref, 4), cp(g_hbm, g_ref, 5), cp(z_hbm, z_ref, 30)]
    cp_w2 = cp(w2t_hbm, w2t_ref, 6)
    cp_x1 = cp(x_hbm.at[:, c0:], x_ref.at[:, c0:], 7)
    cp_kvs = [cp(k_hbm, k_ref, 8), cp(v_hbm, v_ref, 9), cp(sk_hbm, sk_ref, 10)]
    for c in cp_c + [cp_w1, cp_x0] + [cp_w2, cp_x1] + cp_kvs:
        c.start()
    for c in cp_c:
        c.wait()

    sh = sh_ref[...].astype(f32)
    dd = d_ref[...].astype(f32).reshape(1, D)
    p = jnp.concatenate([sh, dd, jnp.zeros((3, D), f32)], axis=0)
    p = jnp.concatenate([p, jnp.zeros((8, 64), f32)], axis=1)
    p = jnp.concatenate([p, jnp.zeros((120, 512), f32)], axis=0)
    pt = p.T
    for j in range(5):
        wb_ref[j] = jnp.broadcast_to(pt[0:D, j:j + 1], (D, 128))

    z = z_ref[0]
    false = t_ref[0:16, 0:128] > 2.0

    def tile(n):
        if isinstance(n, int):
            return slice(128 * n, 128 * (n + 1))
        return pl.ds(pl.multiple_of(128 * n, 128), 128)

    def tree(vals):
        vals = list(vals)
        while len(vals) > 1:
            nxt = [vals[i] + vals[i + 1] for i in range(0, len(vals) - 1, 2)]
            if len(vals) % 2:
                nxt.append(vals[-1])
            vals = nxt
        return vals[0]

    def ln(n):
        x = x_ref[:, tile(n)].astype(f32)
        xv = [x[8 * i:8 * i + 8] for i in range(NG)]
        m = jnp.sum(tree(xv), axis=0, keepdims=True) * (1.0 / D)
        xc = [v - m for v in xv]
        var = jnp.sum(tree([v * v for v in xc]), axis=0, keepdims=True) * (1.0 / D)
        r = 0.5 * jax.lax.rsqrt(var + 1e-5)
        xh = jnp.concatenate([v * r for v in xc], axis=0).astype(bf16)
        xn_ref[:, tile(n)] = xh
        return xh

    def e_group(g):
        rs = slice(8 * g, 8 * g + 8)
        xr = [xh_ref[a, 0, rs] for a in range(NB)]
        xi = [xh_ref[a, 1, rs] for a in range(NB)]
        xs = [xh_ref[a, 2, rs] for a in range(NB)]
        kr = [kh_ref[c, 0, rs] for c in range(NB)]
        kd = [kh_ref[c, 1, rs] for c in range(NB)]
        ks = [kh_ref[c, 2, rs] for c in range(NB)]
        outs = []
        pre = pim = None
        for s in range(NB):
            s1 = s2 = s3 = None
            for a in range(s + 1):
                c = s - a
                t1, t2, t3 = kr[c] * xs[a], kd[c] * xr[a], ks[c] * xi[a]
                s1 = t1 if s1 is None else s1 + t1
                s2 = t2 if s2 is None else s2 + t2
                s3 = t3 if s3 is None else s3 + t3
            re, im = s1 - s3, s1 + s2
            if pre is None:
                wr, wi = re, im
            else:
                wr, wi = re + pim, im - pre
            pre, pim = re, im
            wv_ref[s, 0, rs] = wr
            wv_ref[s, 1, rs] = wi
            outs.append((wr, wi))
        return outs

    cum = np.cumsum(np.arange(1, NB + 1)) / 136.0
    state = dict(g=0, pending=[], t=0.0)

    def e_fill(t_end):
        while TIES and state['g'] < NG and state['g'] * EGAP < t_end:
            g = state['g']
            outs = e_group(g)
            for s, (wr, wi) in enumerate(outs):
                tt = (g + cum[s]) * EGAP
                state['pending'].append((tt, wr))
                state['pending'].append((tt, wi))
            state['g'] += 1

    def tie_lhs(ref, c0_, nrow, slots, t0, dur, kt_w):
        e_fill(t0 + dur)
        pend = state['pending']
        if not pend:
            state['t'] = t0 + dur
            return ref[:, c0_:c0_ + sum(kt_w)]
        assign = {}
        slots = sorted(slots)
        si = 0
        rest = []
        for (tt, v) in pend:
            if tt >= t0 + dur - 8 and state['g'] < NG or si >= len(slots):
                rest.append((tt, v))
                continue
            while si < len(slots) - 1 and t0 + slots[si][0] < tt:
                si += 1
            assign[slots[si][1:]] = v
            si += 1
        state['pending'] = rest
        state['t'] = t0 + dur
        nkt = len(kt_w)
        cols = []
        for t in range(nkt):
            lo = c0_ + sum(kt_w[:t])
            if not any(k[1] == t for k in assign):
                cols.append(ref[:, lo:lo + kt_w[t]])
                continue
            rows = []
            r = 0
            tied = sorted(k[0] for k in assign if k[1] == t)
            for rt in tied:
                if rt > r:
                    rows.append(ref[16 * r:16 * rt, lo:lo + kt_w[t]])
                base = ref[16 * rt:16 * rt + 16, lo:lo + kt_w[t]]
                rows.append(jnp.where(false, pltpu.bitcast(assign[(rt, t)], bf16), base))
                r = rt + 1
            if 16 * r < nrow:
                rows.append(ref[16 * r:nrow, lo:lo + kt_w[t]])
            cols.append(jnp.concatenate(rows, axis=0))
        return jnp.concatenate(cols, axis=1)

    slots1 = [(16 * r, r, t) for r in range(F // 16) for t in range(3)]
    slots2 = [(448 * (t // 4) + 16 * r, r, t) for r in range(D // 16) for t in range(12)]
    slots2 += [(1344 + 16 * (r % 14), r, t) for r in range(D // 16) for t in (12, 13)]

    def mm1(n, xh, tied):
        lhs = tie_lhs(w1t_ref, 0, F, slots1, state['t'], 1792, [128, 128, 128, 64]) if tied else w1t_ref[...]
        h = jnp.dot(lhs, xh, preferred_element_type=f32)
        h_ref[:, tile(n)] = (h + h * jnp.tanh(h)).astype(bf16)

    slots2a = [(16 * r, r, t) for r in range(D // 16) for t in range(4)]
    slots2b = [(16 * (r % 14), r, t) for r in range(D // 16) for t in range(2)]

    def mm2(n, tied):
        acc = None
        for q in range(4):
            lo, hi = 512 * q, min(512 * q + 512, F)
            tied = tied and TIES and (state['g'] < NG or state['pending'])
            if tied:
                lhs = tie_lhs(w2t_ref, lo, D, slots2a if q < 3 else slots2b, state['t'], 448 if q < 3 else 224, [128] * ((hi - lo) // 128))
            else:
                lhs = w2t_ref[:, lo:hi]
            r = jnp.dot(lhs, h_ref[lo:hi, tile(n)], preferred_element_type=f32)
            acc = r if acc is None else acc + r
        acc_ref[:, tile(n)] = acc

    cp_w1.wait()
    cp_x0.wait()
    w1t_ref[...] = w1_ref[...].T
    if LOOPS & 1:
        @pl.loop(0, X0)
        def _(n):
            mm1(n, ln(n), False)
    else:
        for n in range(X0):
            mm1(n, ln(n), False)
    cp_w2.wait()
    cp_x1.wait()
    if LOOPS & 2:
        @pl.loop(0, X0)
        def _(n):
            mm2(n, False)
    else:
        for n in range(X0):
            mm2(n, False)
    for n in range(X0, N_PRE):
        mm1(n, ln(n), False)
        mm2(n, False)
    for c in cp_kvs:
        c.wait()

    lane = jax.lax.broadcasted_iota(jnp.int32, (D // 2, 128), 1)
    prev = [jnp.zeros((D // 2, 128), u32)] * 3
    T = t_ref[...]
    for a in range(NB):
        kt = pltpu.bitcast(k_ref[:, tile(a)], u32)
        acc = pltpu.bitcast(kt, bf16).astype(f32) * wb_ref[0]
        cur = []
        for j in range(1, 4):
            r = pltpu.roll(kt, j, 1)
            cur.append(r)
            sel = jnp.where(lane < j, prev[j - 1], r)
            acc = acc + pltpu.bitcast(sel, bf16).astype(f32) * wb_ref[j]
        prev = cur
        kv = (acc * v_ref[:, tile(a)].astype(f32)).astype(bf16)
        lhs = jnp.concatenate([kv, sk_ref[:, tile(a)]], axis=0)
        r = jnp.dot(lhs, T, preferred_element_type=f32)
        xr, xi = r[:D, :128], r[:D, 128:]
        xh_ref[a + z, 0, 0:D] = xr
        xh_ref[a + z, 1, 0:D] = xi
        xh_ref[a + z, 2, 0:D] = xr + xi
        kr, ki = r[D:, :128], r[D:, 128:]
        if a == 0:
            kr = kr + wb_ref[4]
        kh_ref[a + z, 0, 0:D] = kr
        kh_ref[a + z, 1, 0:D] = ki - kr
        kh_ref[a + z, 2, 0:D] = kr + ki

    G = g_ref[...]
    cps = []

    def inv_final(s):
        lhs = jnp.concatenate([wv_ref[s, 0].astype(bf16), wv_ref[s, 1].astype(bf16)], axis=1)
        y = jnp.dot(lhs, G, preferred_element_type=f32)
        o = x_ref[:, tile(s)].astype(f32) + xn_ref[:, tile(s)].astype(f32) * y + acc_ref[:, tile(s)]
        o_ref[:, tile(s)] = o.astype(bf16)
        if (s + 1) % OG == 0:
            cs = slice(128 * (s + 1 - OG), 128 * (s + 1))
            c = cp(o_ref.at[:, cs], o_hbm.at[:, cs], 11 + s)
            c.start()
            cps.append(c)

    done_inv = False
    if not TIES:
        for g in range(NG):
            e_group(g)
    for n in range(N_PRE, NB):
        tied = TIES and (state['g'] < NG or state['pending'])
        mm1(n, ln(n), tied)
        tied = TIES and (state['g'] < NG or state['pending'])
        mm2(n, tied)
        if done_inv:
            inv_final(n)
        elif state['g'] == NG and not state['pending'] or not TIES and n == 11:
            for s in range(n + 1):
                inv_final(s)
            done_inv = True
    assert done_inv
    for c in cps:
        c.wait()


def fn(A_q, A_k, A_v, A_shift_k, A_ssm_k, A_ssm_D, B_x, B_w1, B_w2):
    T, G = _consts()
    f32, bf16 = jnp.float32, jnp.bfloat16
    hbm = pl.BlockSpec(memory_space=pl.ANY)
    out = pl.pallas_call(
        kernel,
        out_shape=jax.ShapeDtypeStruct((D, S), bf16),
        in_specs=[hbm] * 11,
        out_specs=hbm,
        scratch_shapes=[
            pltpu.VMEM((D, S), bf16), pltpu.VMEM((D, S), bf16), pltpu.VMEM((D, S), bf16),
            pltpu.VMEM((4, D), bf16), pltpu.VMEM((D, S), bf16), pltpu.VMEM((D,), bf16),
            pltpu.VMEM((D, F), bf16), pltpu.VMEM((D, F), bf16),
            pltpu.VMEM((128, 256), bf16), pltpu.VMEM((256, 128), bf16),
            pltpu.VMEM((D, S), bf16),
            pltpu.VMEM((F, D), bf16),
            pltpu.VMEM((D, S), bf16),
            pltpu.VMEM((5, D, 128), f32),
            pltpu.VMEM((F, S), bf16),
            pltpu.VMEM((NB, 3, D + 8, 128), f32),
            pltpu.VMEM((NB, 3, D + 8, 128), f32),
            pltpu.VMEM((NB, 2, D, 128), f32),
            pltpu.VMEM((D, S), f32),
            pltpu.SMEM((8,), jnp.int32),
            pltpu.SemaphoreType.DMA((32,)),
        ],
        compiler_params=pltpu.CompilerParams(vmem_limit_bytes=120 * 2**20),
    )(A_q[0].T, A_k[0].T, A_v[0].T, A_shift_k.T, A_ssm_k, A_ssm_D, B_w1, B_w2.T, T, G, np.array([0, 7, 3, 9, 1, 1, 4, 2], np.int32))
    return out.T[None]


@jax.jit
def pallas_parallel_sum__ssm_conv_h3__dense_activation_silu__prompt_kernel(
    A_q, A_k, A_v, A_shift_k, A_ssm_k, A_ssm_D, B_x, B_w1, B_w2):
    return fn(A_q, A_k, A_v, A_shift_k, A_ssm_k, A_ssm_D, B_x, B_w1, B_w2)
```

```python
import numpy as np
import jax
import jax.numpy as jnp
import jax.experimental.pallas as pl
import jax.experimental.pallas.tpu as pltpu

S, D, F = 2048, 448, 1792
NB = S // 128
NG = D // 8

EGAP = 448
N_PRE = 6
LNTIE = 1
U32 = 0
LN_T0 = 300
LN_T1 = 40
EDYN = 0
VF = 1
LN1TIE = 1
XS = 0
X00 = 1
W3Q = 2
PAIR = 1
LN_DT = 16
W1CH = [0,512,1792]
W1AT = 3
WVDYN = 0
SC = 0
import contextlib
def scope(name):
    return jax.named_scope(name) if SC else contextlib.nullcontext()


def _consts():
    b = np.arange(128, dtype=np.float64)[:, None]
    f = np.arange(128, dtype=np.float64)[None, :]
    th = 2.0 * np.pi * b * (f - 0.25) / 128.0
    T = np.concatenate([np.cos(th), -np.sin(th)], axis=1)
    G = T.T / 64.0
    return T.astype(jnp.bfloat16), G.astype(jnp.bfloat16)


def kernel(x_hbm, k_hbm, v_hbm, sh_hbm, sk_hbm, d_hbm, w1_hbm, w2t_hbm, t_hbm, g_hbm, z_hbm, o_hbm,
           x_ref, k_ref, v_ref, sh_ref, sk_ref, d_ref, w1_ref, w2t_ref, t_ref, g_ref, o_ref,
           w1t_ref, w2p_ref, xn_ref, wb_ref, h_ref, xh_ref, kh_ref, wv_ref, acc_ref, z_ref, sems):
    f32, bf16, u32 = jnp.float32, jnp.bfloat16, jnp.uint32
    nsem = [0]

    def cp(src, dst):
        nsem[0] += 1
        return pltpu.make_async_copy(src, dst, sems.at[nsem[0] - 1])

    def cols(ref, lo, hi):
        return ref.at[:, lo:hi]

    cp_x0 = cp(cols(x_hbm, 0, 128 if X00 else 512), cols(x_ref, 0, 128 if X00 else 512))
    cp_x0b = cp(cols(x_hbm, 128, 512), cols(x_ref, 128, 512)) if X00 else None
    cp_c = [cp(sh_hbm, sh_ref), cp(d_hbm, d_ref), cp(t_hbm, t_ref), cp(g_hbm, g_ref), cp(z_hbm, z_ref)]
    cp_w1 = [cp(cols(w1_hbm, lo, hi), cols(w1_ref, lo, hi)) for lo, hi in zip(W1CH[:-1], W1CH[1:])]
    cp_w2 = cp(w2t_hbm, w2t_ref)
    cp_x1 = cp(cols(x_hbm, 512, 1024), cols(x_ref, 512, 1024))
    cp_rest = [cp(cols(x_hbm, 1024, S), cols(x_ref, 1024, S)), cp(k_hbm, k_ref), cp(v_hbm, v_ref), cp(sk_hbm, sk_ref)]
    cp_z = cp_c.pop()
    for c in [cp_z, cp_x0, cp_w1[0]] + ([cp_x0b] if X00 else []) + cp_w1[1:] + cp_c + [cp_w2, cp_x1] + cp_rest:
        c.start()

    def tile(n):
        if isinstance(n, int):
            return slice(128 * n, 128 * (n + 1))
        return pl.ds(pl.multiple_of(128 * n, 128), 128)

    def tree(vals):
        vals = list(vals)
        while len(vals) > 1:
            nxt = [vals[i] + vals[i + 1] for i in range(0, len(vals) - 1, 2)]
            if len(vals) % 2:
                nxt.append(vals[-1])
            vals = nxt
        return vals[0]

    def ln(n):
        x = x_ref[:, tile(n)].astype(f32)
        xv = [x[8 * i:8 * i + 8] for i in range(NG)]
        m = jnp.sum(tree(xv), axis=0, keepdims=True) * (1.0 / D)
        xc = [v - m for v in xv]
        var = jnp.sum(tree([v * v for v in xc]), axis=0, keepdims=True) * (1.0 / D)
        r = 0.5 * jax.lax.rsqrt(var + 1e-5)
        parts = [jnp.concatenate([xc[2 * i] * r, xc[2 * i + 1] * r], axis=0).astype(bf16) for i in range(NG // 2)]
        xh = jnp.concatenate(parts, axis=0)
        xn_ref[:, tile(n)] = xh
        return xh, parts

    st = dict(g=0, pending=[], t=0.0, e0=None, false=None)

    def load_lhs(ref, r0, r1, c0, c1):
        if ref.dtype == u32:
            return pltpu.bitcast(ref[r0 // 2:r1 // 2, c0:c1], bf16)
        return ref[r0:r1, c0:c1]

    cum = np.cumsum(np.arange(1, NB + 1)) / 136.0

    def e_group(g):
        rs = slice(8 * g, 8 * g + 8)
        ez = z if EDYN else 0
        xr = [xh_ref[a + ez, 0, rs] for a in range(NB)]
        xi = [xh_ref[a + ez, 1, rs] for a in range(NB)]
        xs = [xh_ref[a + ez, 2, rs] for a in range(NB)] if XS else [xr[a] + xi[a] for a in range(NB)]
        kr = [kh_ref[c + ez, 0, rs] for c in range(NB)]
        kd = [kh_ref[c + ez, 1, rs] for c in range(NB)]
        ks = [kh_ref[c + ez, 2, rs] for c in range(NB)]
        outs = []
        pre = pim = None
        for s in range(NB):
            s1 = s2 = s3 = None
            for a in range(s + 1):
                c = s - a
                t1, t2, t3 = kr[c] * xs[a], kd[c] * xr[a], ks[c] * xi[a]
                s1 = t1 if s1 is None else s1 + t1
                s2 = t2 if s2 is None else s2 + t2
                s3 = t3 if s3 is None else s3 + t3
            re, im = s1 - s3, s1 + s2
            if pre is None:
                wr, wi = re, im
            else:
                wr, wi = re + pim, im - pre
            pre, pim = re, im
            zz = z if WVDYN else 0
            wv_ref[s + zz, 0, rs] = wr
            wv_ref[s + zz, 1, rs] = wi
            outs.append((wr, wi))
        return outs

    def e_fill(t_end):
        while st['e0'] is not None and st['g'] < NG and st['e0'] + st['g'] * EGAP < t_end:
            g = st['g']
            for s, (wr, wi) in enumerate(e_group(g)):
                tt = st['e0'] + (g + cum[s]) * EGAP
                st['pending'].append((tt, pltpu.bitcast(wr, bf16)))
                st['pending'].append((tt, pltpu.bitcast(wi, bf16)))
            st['g'] += 1

    def e_active():
        return st['e0'] is not None and st['g'] < NG

    def tie_lhs(ref, r0_, c0_, nrow, slots, dur, kt_w):
        t0 = st['t']
        st['t'] = t0 + dur
        e_fill(t0 + dur)
        pend = sorted(st['pending'], key=lambda p: p[0])
        if not pend:
            return load_lhs(ref, r0_, r0_ + nrow, c0_, c0_ + sum(kt_w))
        assign, rest, si = {}, [], 0
        slots = sorted(slots)
        for (tt, v) in pend:
            if (tt >= t0 + dur - 8 and not st.get('flush')) or si >= len(slots):
                rest.append((tt, v))
                continue
            while si < len(slots) - 1 and t0 + slots[si][0] < tt:
                si += 1
            assign[slots[si][1:]] = v
            si += 1
        st['pending'] = rest
        colsl = []
        for t in range(len(kt_w)):
            lo = c0_ + sum(kt_w[:t])
            hi = lo + kt_w[t]
            rows, r = [], 0
            for rt in sorted(k[0] for k in assign if k[1] == t):
                if rt > r:
                    rows.append(load_lhs(ref, r0_ + 16 * r, r0_ + 16 * rt, lo, hi))
                base = load_lhs(ref, r0_ + 16 * rt, r0_ + 16 * rt + 16, lo, hi)
                rows.append(jnp.where(st['false'], assign[(rt, t)], base))
                r = rt + 1
            if 16 * r < nrow:
                rows.append(load_lhs(ref, r0_ + 16 * r, r0_ + nrow, lo, hi))
            colsl.append(rows[0] if len(rows) == 1 else jnp.concatenate(rows, axis=0))
        return jnp.concatenate(colsl, axis=1)

    def ln_tied(n, t_start):
        xh, parts = ln(n)
        for i, pz in enumerate(parts):
            st['pending'].append((t_start + LN_DT * i, pz))
        return xh

    def slots1(nrow):
        return [(16 * r, r, t) for r in range(nrow // 16) for t in range(3)]
    slots2a = [(16 * r, r, t) for r in range(D // 16) for t in range(4)]
    slots2b = [(16 * (r % 14), r, t) for r in range(D // 16) for t in range(2)]

    def mm1(n, xh, lo=0, hi=F):
        lhs = tie_lhs(w1t_ref, lo, 0, hi - lo, slots1(hi - lo), hi - lo, [128, 128, 128, 64])
        h = jnp.dot(lhs, xh, preferred_element_type=f32)
        h_ref[lo:hi, tile(n)] = (h + h * jnp.tanh(h)).astype(bf16)

    slots2c = [(16 * r, r, t) for r in range(D // 16) for t in range(2)]
    held = {}

    def mm2(n, ln_next=None, raw=False, repack=False, pair=False, hook=None):
        if ln_next is not None:
            ln_tied(ln_next, st['t'] + LN_T0)
        acc = None
        src = w2t_ref if (raw or not U32) else w2p_ref
        for q in range(4):
            lo, hi = 512 * q, min(512 * q + 512, F)
            if hook is not None and q == W3Q:
                hook()
            if q == 3 and pair:
                if n % 2 == 0:
                    held[n] = acc
                    return
                lhs = tie_lhs(src, 0, lo, D, slots2c, 448, [128, 128])
                cs2 = slice(128 * (n - 1), 128 * (n + 1))
                r = jnp.dot(lhs, h_ref[lo:hi, cs2], preferred_element_type=f32)
                acc_ref[:, tile(n - 1)] = held.pop(n - 1) + r[:, :128]
                acc_ref[:, tile(n)] = acc + r[:, 128:]
                return
            lhs = tie_lhs(src, 0, lo, D, slots2a if q < 3 else slots2b, 448 if q < 3 else 224, [128] * ((hi - lo) // 128))
            if repack and U32:
                w2p_ref[:, lo:hi] = pltpu.bitcast(lhs, u32)
            r = jnp.dot(lhs, h_ref[lo:hi, tile(n)], preferred_element_type=f32)
            acc = r if acc is None else acc + r
        acc_ref[:, tile(n)] = acc

    def w1_chunk(ci):
        lo, hi = W1CH[ci], W1CH[ci + 1]
        with scope("waitw1_%d" % ci):
            cp_w1[ci].wait()
        wt = w1_ref[:, lo:hi].T
        if U32:
            w1t_ref[lo // 2:hi // 2, :] = pltpu.bitcast(wt, u32)
        else:
            w1t_ref[lo:hi, :] = wt

    with scope("waitx0"):
        cp_z.wait()
        cp_x0.wait()
    z = z_ref[0]
    st['false'] = z_ref[1] < 0
    w1_chunk(0)
    xhs = [ln(0)[0]] + [None] * 3
    nch = len(W1CH) - 1
    for ci in range(nch):
        lo, hi = W1CH[ci], W1CH[ci + 1]
        for n in range(4):
            if n == W1AT and ci + 1 < nch:
                w1_chunk(ci + 1)
            if X00 and ci == 0 and n == 1:
                cp_x0b.wait()
                xhs[1] = ln(1)[0]
            if ci == 0 and n < 3 and not (X00 and n == 0):
                if n + 1 <= W1AT and LN1TIE:
                    xhs[n + 1] = ln_tied(n + 1, st['t'] + LN_T1)
                else:
                    xhs[n + 1] = ln(n + 1)[0]
                st['flush'] = True
            mm1(n, xhs[n] if ci == 0 else xn_ref[:, tile(n)], lo, hi)
            st['flush'] = False

    with scope("wait2"):
        for c in cp_c + [cp_w2, cp_x1]:
            c.wait()
    if VF:
        st['false'] = t_ref[0:16, 0:128] > 2.0

    @pl.loop(0, 4)
    def _(n):
        mm2(n, (n + 4) if LNTIE else None, raw=True)
        if not LNTIE:
            ln(n + 4)
        assert not st['pending']

    sh = sh_ref[...].astype(f32)
    dd = d_ref[...].astype(f32).reshape(1, D)
    p = jnp.concatenate([sh, dd, jnp.zeros((3, D), f32)], axis=0)
    p = jnp.concatenate([p, jnp.zeros((8, 64), f32)], axis=1)
    p = jnp.concatenate([p, jnp.zeros((120, 512), f32)], axis=0)
    pt = p.T
    for j in range(5):
        wb_ref[j] = jnp.broadcast_to(pt[0:D, j:j + 1], (D, 128))

    for n in range(4, N_PRE):
        mm1(n, xn_ref[:, tile(n)])
        def wait3():
            with scope("wait3"):
                for c in cp_rest:
                    c.wait()
        mm2(n, raw=(n == 4), repack=(n == 4), pair=PAIR and n >= 6, hook=wait3 if n == N_PRE - 1 else None)

    lane = jax.lax.broadcasted_iota(jnp.int32, (D // 2, 128), 1)
    prev = [jnp.zeros((D // 2, 128), u32)] * 3
    T = t_ref[...]
    for a in range(NB):
        kt = pltpu.bitcast(k_ref[:, tile(a)], u32)
        acc = pltpu.bitcast(kt, bf16).astype(f32) * wb_ref[0]
        cur = []
        for j in range(1, 4):
            r = pltpu.roll(kt, j, 1)
            cur.append(r)
            sel = jnp.where(lane < j, prev[j - 1], r)
            acc = acc + pltpu.bitcast(sel, bf16).astype(f32) * wb_ref[j]
        prev = cur
        kv = (acc * v_ref[:, tile(a)].astype(f32)).astype(bf16)
        lhs = jnp.concatenate([kv, sk_ref[:, tile(a)]], axis=0)
        r = jnp.dot(lhs, T, preferred_element_type=f32)
        xr, xi = r[:D, :128], r[:D, 128:]
        xh_ref[a + z, 0, 0:D] = xr
        xh_ref[a + z, 1, 0:D] = xi
        if XS:
            xh_ref[a + z, 2, 0:D] = xr + xi
        kr, ki = r[D:, :128], r[D:, 128:]
        if a == 0:
            kr = kr + wb_ref[4]
        kh_ref[a + z, 0, 0:D] = kr
        kh_ref[a + z, 1, 0:D] = ki - kr
        kh_ref[a + z, 2, 0:D] = kr + ki

    G = g_ref[...]
    cps = []

    def inv_final(s):
        lhs = jnp.concatenate([wv_ref[s, 0, 0:D].astype(bf16), wv_ref[s, 1, 0:D].astype(bf16)], axis=1)
        y = jnp.dot(lhs, G, preferred_element_type=f32)
        o = x_ref[:, tile(s)].astype(f32) + xn_ref[:, tile(s)].astype(f32) * y + acc_ref[:, tile(s)]
        o_ref[:, tile(s)] = o.astype(bf16)
        c = cp(o_ref.at[:, tile(s)], o_hbm.at[:, tile(s)])
        c.start()
        cps.append(c)

    st['e0'] = st['t']
    done_inv = False
    have_ln = 8
    for n in range(N_PRE, NB):
        if n >= have_ln:
            xh = ln(n)[0]
            have_ln = n + 1
        else:
            xh = xn_ref[:, tile(n)]
        mm1(n, xh)
        nxt = None
        if LNTIE and n + 1 < NB and n + 1 >= have_ln:
            nxt = n + 1
            have_ln = n + 2
        mm2(n, nxt, pair=PAIR)
        if PAIR and n % 2 == 0:
            continue
        if done_inv:
            for s in range(n - 1 if PAIR else n, n + 1):
                inv_final(s)
        elif st['g'] == NG and not st['pending']:
            for s in range(n + 1):
                inv_final(s)
            done_inv = True
    assert done_inv
    with scope("wait4"):
        for c in cps:
            c.wait()


def fn(A_q, A_k, A_v, A_shift_k, A_ssm_k, A_ssm_D, B_x, B_w1, B_w2):
    T, G = _consts()
    f32, bf16, u32 = jnp.float32, jnp.bfloat16, jnp.uint32
    hbm = pl.BlockSpec(memory_space=pl.ANY)
    out = pl.pallas_call(
        kernel,
        out_shape=jax.ShapeDtypeStruct((D, S), bf16),
        in_specs=[hbm] * 11,
        out_specs=hbm,
        scratch_shapes=[
            pltpu.VMEM((D, S), bf16), pltpu.VMEM((D, S), bf16), pltpu.VMEM((D, S), bf16),
            pltpu.VMEM((4, D), bf16), pltpu.VMEM((D, S), bf16), pltpu.VMEM((D,), bf16),
            pltpu.VMEM((D, F), bf16), pltpu.VMEM((D, F), bf16),
            pltpu.VMEM((128, 256), bf16), pltpu.VMEM((256, 128), bf16),
            pltpu.VMEM((D, S), bf16),
            pltpu.VMEM((F // 2, D), u32) if U32 else pltpu.VMEM((F, D), bf16),
            pltpu.VMEM((D // 2, F), u32),
            pltpu.VMEM((D, S), bf16),
            pltpu.VMEM((5, D, 128), f32),
            pltpu.VMEM((F, S), bf16),
            pltpu.VMEM((NB, 3, D + 8, 128), f32),
            pltpu.VMEM((NB, 3, D + 8, 128), f32),
            pltpu.VMEM((NB, 2, D + 8, 128), f32),
            pltpu.VMEM((D, S), f32),
            pltpu.SMEM((8,), jnp.int32),
            pltpu.SemaphoreType.DMA((40,)),
        ],
        compiler_params=pltpu.CompilerParams(vmem_limit_bytes=120 * 2**20),
    )(A_q[0].T, A_k[0].T, A_v[0].T, A_shift_k.T, A_ssm_k, A_ssm_D, B_w1, B_w2.T, T, G,
      np.array([0, 7, 3, 9, 1, 1, 4, 2], np.int32))
    return out.T[None]


@jax.jit
def pallas_parallel_sum__ssm_conv_h3__dense_activation_silu__prompt_kernel(
    A_q, A_k, A_v, A_shift_k, A_ssm_k, A_ssm_D, B_x, B_w1, B_w2):
    return fn(A_q, A_k, A_v, A_shift_k, A_ssm_k, A_ssm_D, B_x, B_w1, B_w2)
```

```python
import numpy as np
import jax
import jax.numpy as jnp
import jax.experimental.pallas as pl
import jax.experimental.pallas.tpu as pltpu

S, D, F = 2048, 448, 1792
NB = S // 128
NG = D // 8

EGAP = 448
N_PRE = 6
LNTIE = 1
U32 = 0
LN_T0 = 300
LN_T1 = 40
EDYN = 0
VF = 1
LN1TIE = 1
EARLY = 1
LNM = 0
LNM_T = 250
LP = 2
L1 = 0
L2 = 0
XS = 0
X00 = 1
W3Q = 2
PAIR = 1
LN_DT = 16
W1CH = [0,512,1792]
W1AT = 3
WVDYN = 0
SC = 0
import contextlib
def scope(name):
    return jax.named_scope(name) if SC else contextlib.nullcontext()


def _consts():
    b = np.arange(128, dtype=np.float64)[:, None]
    f = np.arange(128, dtype=np.float64)[None, :]
    th = 2.0 * np.pi * b * (f - 0.25) / 128.0
    T = np.concatenate([np.cos(th), -np.sin(th)], axis=1)
    G = T.T / 64.0
    return T.astype(jnp.bfloat16), G.astype(jnp.bfloat16)


def kernel(x_hbm, k_hbm, v_hbm, sh_hbm, sk_hbm, d_hbm, w1_hbm, w2t_hbm, t_hbm, g_hbm, z_hbm, o_hbm,
           x_ref, k_ref, v_ref, sh_ref, sk_ref, d_ref, w1_ref, w2t_ref, t_ref, g_ref, o_ref,
           w1t_ref, w2p_ref, xn_ref, wb_ref, h_ref, xh_ref, kh_ref, wv_ref, acc_ref, z_ref, sems):
    f32, bf16, u32 = jnp.float32, jnp.bfloat16, jnp.uint32
    nsem = [0]

    def cp(src, dst):
        nsem[0] += 1
        return pltpu.make_async_copy(src, dst, sems.at[nsem[0] - 1])

    def cols(ref, lo, hi):
        return ref.at[:, lo:hi]

    cp_x0 = cp(cols(x_hbm, 0, 128 if X00 else 512), cols(x_ref, 0, 128 if X00 else 512))
    cp_x0b = cp(cols(x_hbm, 128, 512), cols(x_ref, 128, 512)) if X00 else None
    cp_c = [cp(sh_hbm, sh_ref), cp(d_hbm, d_ref), cp(t_hbm, t_ref), cp(g_hbm, g_ref), cp(z_hbm, z_ref)]
    cp_w1 = [cp(cols(w1_hbm, lo, hi), cols(w1_ref, lo, hi)) for lo, hi in zip(W1CH[:-1], W1CH[1:])]
    cp_w2 = cp(w2t_hbm, w2t_ref)
    cp_x1 = cp(cols(x_hbm, 512, 1024), cols(x_ref, 512, 1024))
    cp_rest = [cp(cols(x_hbm, 1024, S), cols(x_ref, 1024, S)), cp(k_hbm, k_ref), cp(v_hbm, v_ref), cp(sk_hbm, sk_ref)]
    cp_z = cp_c.pop()
    for c in [cp_z, cp_x0, cp_w1[0]] + ([cp_x0b] if X00 else []) + cp_w1[1:] + cp_c + [cp_w2, cp_x1] + cp_rest:
        c.start()

    def tile(n):
        if isinstance(n, int):
            return slice(128 * n, 128 * (n + 1))
        return pl.ds(pl.multiple_of(128 * n, 128), 128)

    def tree(vals):
        vals = list(vals)
        while len(vals) > 1:
            nxt = [vals[i] + vals[i + 1] for i in range(0, len(vals) - 1, 2)]
            if len(vals) % 2:
                nxt.append(vals[-1])
            vals = nxt
        return vals[0]

    def ln(n):
        x = x_ref[:, tile(n)].astype(f32)
        xv = [x[8 * i:8 * i + 8] for i in range(NG)]
        m = jnp.sum(tree(xv), axis=0, keepdims=True) * (1.0 / D)
        xc = [v - m for v in xv]
        var = jnp.sum(tree([v * v for v in xc]), axis=0, keepdims=True) * (1.0 / D)
        r = 0.5 * jax.lax.rsqrt(var + 1e-5)
        parts = [jnp.concatenate([xc[2 * i] * r, xc[2 * i + 1] * r], axis=0).astype(bf16) for i in range(NG // 2)]
        xh = jnp.concatenate(parts, axis=0)
        xn_ref[:, tile(n)] = xh
        st['lnstat'] = (m, r)
        return xh, parts

    st = dict(g=0, pending=[], t=0.0, e0=None, false=None)

    def load_lhs(ref, r0, r1, c0, c1):
        if ref.dtype == u32:
            return pltpu.bitcast(ref[r0 // 2:r1 // 2, c0:c1], bf16)
        return ref[r0:r1, c0:c1]

    cum = np.cumsum(np.arange(1, NB + 1)) / 136.0

    def e_group(g):
        rs = slice(8 * g, 8 * g + 8)
        ez = z if EDYN else 0
        xr = [xh_ref[a + ez, 0, rs] for a in range(NB)]
        xi = [xh_ref[a + ez, 1, rs] for a in range(NB)]
        xs = [xh_ref[a + ez, 2, rs] for a in range(NB)] if XS else [xr[a] + xi[a] for a in range(NB)]
        kr = [kh_ref[c + ez, 0, rs] for c in range(NB)]
        kd = [kh_ref[c + ez, 1, rs] for c in range(NB)]
        ks = [kh_ref[c + ez, 2, rs] for c in range(NB)]
        outs = []
        pre = pim = None
        for s in range(NB):
            s1 = s2 = s3 = None
            for a in range(s + 1):
                c = s - a
                t1, t2, t3 = kr[c] * xs[a], kd[c] * xr[a], ks[c] * xi[a]
                s1 = t1 if s1 is None else s1 + t1
                s2 = t2 if s2 is None else s2 + t2
                s3 = t3 if s3 is None else s3 + t3
            re, im = s1 - s3, s1 + s2
            if pre is None:
                wr, wi = re, im
            else:
                wr, wi = re + pim, im - pre
            pre, pim = re, im
            zz = z if WVDYN else 0
            wv_ref[s + zz, 0, rs] = wr
            wv_ref[s + zz, 1, rs] = wi
            outs.append((wr, wi))
        return outs

    def e_fill(t_end):
        while st['e0'] is not None and st['g'] < NG and st['e0'] + st['g'] * EGAP < t_end:
            g = st['g']
            for s, (wr, wi) in enumerate(e_group(g)):
                tt = st['e0'] + (g + cum[s]) * EGAP
                st['pending'].append((tt, pltpu.bitcast(wr, bf16)))
                st['pending'].append((tt, pltpu.bitcast(wi, bf16)))
            st['g'] += 1

    def e_active():
        return st['e0'] is not None and st['g'] < NG

    def tie_lhs(ref, r0_, c0_, nrow, slots, dur, kt_w):
        t0 = st['t']
        st['t'] = t0 + dur
        e_fill(t0 + dur)
        pend = sorted(st['pending'], key=lambda p: p[0])
        if not pend:
            return load_lhs(ref, r0_, r0_ + nrow, c0_, c0_ + sum(kt_w))
        assign, rest, si = {}, [], 0
        slots = sorted(slots)
        for (tt, v) in pend:
            if (tt >= t0 + dur - 8 and not st.get('flush')) or si >= len(slots):
                rest.append((tt, v))
                continue
            while si < len(slots) - 1 and t0 + slots[si][0] < tt:
                si += 1
            assign[slots[si][1:]] = v
            si += 1
        st['pending'] = rest
        colsl = []
        for t in range(len(kt_w)):
            lo = c0_ + sum(kt_w[:t])
            hi = lo + kt_w[t]
            rows, r = [], 0
            for rt in sorted(k[0] for k in assign if k[1] == t):
                if rt > r:
                    rows.append(load_lhs(ref, r0_ + 16 * r, r0_ + 16 * rt, lo, hi))
                base = load_lhs(ref, r0_ + 16 * rt, r0_ + 16 * rt + 16, lo, hi)
                rows.append(jnp.where(st['false'], assign[(rt, t)], base))
                r = rt + 1
            if 16 * r < nrow:
                rows.append(load_lhs(ref, r0_ + 16 * r, r0_ + nrow, lo, hi))
            colsl.append(rows[0] if len(rows) == 1 else jnp.concatenate(rows, axis=0))
        return jnp.concatenate(colsl, axis=1)

    def ln_tied(n, t_start):
        xh, parts = ln(n)
        if LNM:
            m_, r_ = st['lnstat']
            st['pending'].append((t_start - LNM_T, pltpu.bitcast(jnp.broadcast_to(m_, (8, 128)), bf16)))
            st['pending'].append((t_start - LNM_T // 3, pltpu.bitcast(jnp.broadcast_to(r_, (8, 128)), bf16)))
        for i, pz in enumerate(parts):
            st['pending'].append((t_start + LN_DT * i, pz))
        return xh

    def slots1(nrow):
        return [(16 * r, r, t) for r in range(nrow // 16) for t in range(3)]
    slots2a = [(16 * r, r, t) for r in range(D // 16) for t in range(4)]
    slots2b = [(16 * (r % 14), r, t) for r in range(D // 16) for t in range(2)]

    def mm1(n, xh, lo=0, hi=F):
        lhs = tie_lhs(w1t_ref, lo, 0, hi - lo, slots1(hi - lo), hi - lo, [128, 128, 128, 64])
        h = jnp.dot(lhs, xh, preferred_element_type=f32)
        h_ref[lo:hi, tile(n)] = (h + h * jnp.tanh(h)).astype(bf16)

    slots2c = [(16 * r, r, t) for r in range(D // 16) for t in range(2)]
    held = {}

    def mm2(n, ln_next=None, raw=False, repack=False, pair=False, hook=None):
        if ln_next is not None:
            ln_tied(ln_next, st['t'] + LN_T0)
        acc = None
        src = w2t_ref if (raw or not U32) else w2p_ref
        for q in range(4):
            lo, hi = 512 * q, min(512 * q + 512, F)
            if hook is not None and q == W3Q:
                hook()
            if q == 3 and pair:
                if n % 2 == 0:
                    held[n] = acc
                    return
                lhs = tie_lhs(src, 0, lo, D, slots2c, 448, [128, 128])
                cs2 = slice(128 * (n - 1), 128 * (n + 1))
                r = jnp.dot(lhs, h_ref[lo:hi, cs2], preferred_element_type=f32)
                acc_ref[:, tile(n - 1)] = held.pop(n - 1) + r[:, :128]
                acc_ref[:, tile(n)] = acc + r[:, 128:]
                return
            lhs = tie_lhs(src, 0, lo, D, slots2a if q < 3 else slots2b, 448 if q < 3 else 224, [128] * ((hi - lo) // 128))
            if repack and U32:
                w2p_ref[:, lo:hi] = pltpu.bitcast(lhs, u32)
            r = jnp.dot(lhs, h_ref[lo:hi, tile(n)], preferred_element_type=f32)
            acc = r if acc is None else acc + r
        acc_ref[:, tile(n)] = acc

    def w1_chunk(ci):
        lo, hi = W1CH[ci], W1CH[ci + 1]
        with scope("waitw1_%d" % ci):
            cp_w1[ci].wait()
        wt = w1_ref[:, lo:hi].T
        if U32:
            w1t_ref[lo // 2:hi // 2, :] = pltpu.bitcast(wt, u32)
        else:
            w1t_ref[lo:hi, :] = wt

    with scope("waitx0"):
        cp_z.wait()
        cp_x0.wait()
    z = z_ref[0]
    st['false'] = z_ref[1] < 0
    w1_chunk(0)
    xhs = [ln(0)[0]] + [None] * 3
    nch = len(W1CH) - 1
    for ci in range(nch):
        lo, hi = W1CH[ci], W1CH[ci + 1]
        if L1 and ci == nch - 1:
            @pl.loop(0, 4)
            def _(n):
                mm1(n, xn_ref[:, tile(n)], lo, hi)
            continue
        for n in range(4):
            if n == W1AT and ci + 1 < nch:
                w1_chunk(ci + 1)
            if X00 and ci == 0 and n == 0:
                mid = (lo + hi) // 2
                mm1(0, xhs[0], lo, mid)
                cp_x0b.wait()
                xhs[1] = ln_tied(1, st['t'] + 20)
                st['flush'] = True
                mm1(0, xhs[0], mid, hi)
                st['flush'] = False
                continue
            if ci == 0 and n < 3:
                xhs[n + 1] = ln_tied(n + 1, st['t'] + LNM_T + LN_T1)
                st['flush'] = True
            mm1(n, xhs[n] if ci == 0 else xn_ref[:, tile(n)], lo, hi)
            st['flush'] = False

    with scope("wait2"):
        for c in cp_c + [cp_w2, cp_x1]:
            c.wait()
    if VF:
        st['false'] = t_ref[0:16, 0:128] > 2.0

    if LP == 4:
        @pl.loop(0, 4)
        def _(n):
            mm2(n, n + 4, raw=True)
            assert not st['pending']
    elif LP == 2:
        @pl.loop(0, 2)
        def _(i):
            mm2(2 * i, 2 * i + 4, raw=True)
            mm2(2 * i + 1, 2 * i + 5, raw=True)
            assert not st['pending']
    else:
        for n in range(4):
            mm2(n, n + 4, raw=True, pair=(LP == 0))

    sh = sh_ref[...].astype(f32)
    dd = d_ref[...].astype(f32).reshape(1, D)
    p = jnp.concatenate([sh, dd, jnp.zeros((3, D), f32)], axis=0)
    p = jnp.concatenate([p, jnp.zeros((8, 64), f32)], axis=1)
    p = jnp.concatenate([p, jnp.zeros((120, 512), f32)], axis=0)
    pt = p.T
    for j in range(5):
        wb_ref[j] = jnp.broadcast_to(pt[0:D, j:j + 1], (D, 128))

    def wait3():
        with scope("wait3"):
            for c in cp_rest:
                c.wait()
    if L2:
        @pl.loop(4, N_PRE)
        def _(n):
            mm1(n, xn_ref[:, tile(n)])
            mm2(n)
        wait3()
    else:
        for n in range(4, N_PRE):
            mm1(n, xn_ref[:, tile(n)])
            mm2(n, raw=(n == 4), repack=(n == 4), pair=PAIR and n >= 6, hook=wait3 if n == N_PRE - 1 else None)

    lane = jax.lax.broadcasted_iota(jnp.int32, (D // 2, 128), 1)
    prev = [jnp.zeros((D // 2, 128), u32)] * 3
    T = t_ref[...]
    for a in range(NB):
        kt = pltpu.bitcast(k_ref[:, tile(a)], u32)
        acc = pltpu.bitcast(kt, bf16).astype(f32) * wb_ref[0]
        cur = []
        for j in range(1, 4):
            r = pltpu.roll(kt, j, 1)
            cur.append(r)
            sel = jnp.where(lane < j, prev[j - 1], r)
            acc = acc + pltpu.bitcast(sel, bf16).astype(f32) * wb_ref[j]
        prev = cur
        kv = (acc * v_ref[:, tile(a)].astype(f32)).astype(bf16)
        lhs = jnp.concatenate([kv, sk_ref[:, tile(a)]], axis=0)
        r = jnp.dot(lhs, T, preferred_element_type=f32)
        xr, xi = r[:D, :128], r[:D, 128:]
        xh_ref[a + z, 0, 0:D] = xr
        xh_ref[a + z, 1, 0:D] = xi
        if XS:
            xh_ref[a + z, 2, 0:D] = xr + xi
        kr, ki = r[D:, :128], r[D:, 128:]
        if a == 0:
            kr = kr + wb_ref[4]
        kh_ref[a + z, 0, 0:D] = kr
        kh_ref[a + z, 1, 0:D] = ki - kr
        kh_ref[a + z, 2, 0:D] = kr + ki

    G = g_ref[...]
    cps = []

    ys = {}

    def inv(s):
        lhs = jnp.concatenate([wv_ref[s, 0, 0:D].astype(bf16), wv_ref[s, 1, 0:D].astype(bf16)], axis=1)
        ys[s] = jnp.dot(lhs, G, preferred_element_type=f32)

    def inv_final(s):
        if s not in ys:
            inv(s)
        y = ys.pop(s)
        o = x_ref[:, tile(s)].astype(f32) + xn_ref[:, tile(s)].astype(f32) * y + acc_ref[:, tile(s)]
        o_ref[:, tile(s)] = o.astype(bf16)
        c = cp(o_ref.at[:, tile(s)], o_hbm.at[:, tile(s)])
        c.start()
        cps.append(c)

    st['e0'] = st['t']
    done_inv = False
    have_ln = 8
    for n in range(N_PRE, NB):
        if n >= have_ln:
            xh = ln(n)[0]
            have_ln = n + 1
        else:
            xh = xn_ref[:, tile(n)]
        mm1(n, xh)
        nxt = None
        if LNTIE and n + 1 < NB and n + 1 >= have_ln:
            nxt = n + 1
            have_ln = n + 2
        if EARLY and done_inv and n % 2 == 1:
            inv(n - 1)
            inv(n)
        mm2(n, nxt, pair=PAIR)
        if PAIR and n % 2 == 0:
            continue
        if done_inv:
            for s in range(n - 1 if PAIR else n, n + 1):
                inv_final(s)
        elif st['g'] == NG and not st['pending']:
            for s in range(n + 1):
                inv_final(s)
            done_inv = True
    assert done_inv
    with scope("wait4"):
        for c in cps:
            c.wait()


def fn(A_q, A_k, A_v, A_shift_k, A_ssm_k, A_ssm_D, B_x, B_w1, B_w2):
    T, G = _consts()
    f32, bf16, u32 = jnp.float32, jnp.bfloat16, jnp.uint32
    hbm = pl.BlockSpec(memory_space=pl.ANY)
    out = pl.pallas_call(
        kernel,
        out_shape=jax.ShapeDtypeStruct((D, S), bf16),
        in_specs=[hbm] * 11,
        out_specs=hbm,
        scratch_shapes=[
            pltpu.VMEM((D, S), bf16), pltpu.VMEM((D, S), bf16), pltpu.VMEM((D, S), bf16),
            pltpu.VMEM((4, D), bf16), pltpu.VMEM((D, S), bf16), pltpu.VMEM((D,), bf16),
            pltpu.VMEM((D, F), bf16), pltpu.VMEM((D, F), bf16),
            pltpu.VMEM((128, 256), bf16), pltpu.VMEM((256, 128), bf16),
            pltpu.VMEM((D, S), bf16),
            pltpu.VMEM((F // 2, D), u32) if U32 else pltpu.VMEM((F, D), bf16),
            pltpu.VMEM((D // 2, F), u32),
            pltpu.VMEM((D, S), bf16),
            pltpu.VMEM((5, D, 128), f32),
            pltpu.VMEM((F, S), bf16),
            pltpu.VMEM((NB, 3, D + 8, 128), f32),
            pltpu.VMEM((NB, 3, D + 8, 128), f32),
            pltpu.VMEM((NB, 2, D + 8, 128), f32),
            pltpu.VMEM((D, S), f32),
            pltpu.SMEM((8,), jnp.int32),
            pltpu.SemaphoreType.DMA((40,)),
        ],
        compiler_params=pltpu.CompilerParams(vmem_limit_bytes=120 * 2**20),
    )(A_q[0].T, A_k[0].T, A_v[0].T, A_shift_k.T, A_ssm_k, A_ssm_D, B_w1, B_w2.T, T, G,
      np.array([0, 7, 3, 9, 1, 1, 4, 2], np.int32))
    return out.T[None]


@jax.jit
def pallas_parallel_sum__ssm_conv_h3__dense_activation_silu__prompt_kernel(
    A_q, A_k, A_v, A_shift_k, A_ssm_k, A_ssm_D, B_x, B_w1, B_w2):
    return fn(A_q, A_k, A_v, A_shift_k, A_ssm_k, A_ssm_D, B_x, B_w1, B_w2)
```
